```python
import jax
import jax.numpy as jnp

def _softmax(x, axis=-1):
    return jax.nn.softmax(x, axis=axis)
def _gelu(x):
    return jax.nn.gelu(x, approximate=True)
def _silu(x):
    return jax.nn.silu(x)
def _sigmoid(x):
    return jax.nn.sigmoid(x)
def _layernorm(x, axis=-1, eps=1e-5):
    m = jnp.mean(x, axis=axis, keepdims=True)
    v = jnp.var(x, axis=axis, keepdims=True)
    return (x - m) / jnp.sqrt(v + eps)
def _scatter_add(tgt, idx, src, axis=0):
    return tgt.at[idx].add(src)
def _segment_sum(src, seg, n):
    return jax.ops.segment_sum(src, seg, n)
class _Rng:
    def __init__(self, key):
        self._k = key
    def _next(self):
        self._k, sub = jax.random.split(self._k)
        return sub
    def normal(self, shape):
        return jax.random.normal(self._next(), shape, dtype=jnp.bfloat16)
    def randint(self, lo, hi, shape):
        return jax.random.randint(self._next(), shape, lo, hi, dtype=jnp.int32)
    def uniform(self, shape, lo=0.0, hi=1.0):
        return jax.random.uniform(self._next(), shape, jnp.bfloat16, lo, hi)
    def permutation(self, n):
        return jax.random.permutation(self._next(), n)


kernel_name = 'standalone__channel_attn_se__vision'

def _fwd_setup_inputs():
    _rng = _Rng(jax.random.key(int.from_bytes(__import__("os").urandom(4), "little")))
    _w = (lambda a: (lambda t: t.astype(jnp.bfloat16) if jnp.issubdtype(t.dtype, jnp.floating) else t)(jnp.asarray(a)))
    H = W = 384
    C = 96
    r = max(C // 16, 4)
    return {
        "x": _w((lambda *s: _rng.normal(s) * 0.05)(1, H, W, C)),
        "w_down": _w((lambda *s: _rng.normal(s) * 0.05)(C, r)),
        "w_up": _w((lambda *s: _rng.normal(s) * 0.05)(r, C)),
    }

def _fwd_reference(x, w_down, w_up):
    s = x.mean(axis=(1, 2))
    h = _silu(jnp.einsum('bc,cr->br', s, w_down))
    g = _sigmoid(jnp.einsum('br,rc->bc', h, w_up))
    return x * g[:, None, None, :]


def setup_inputs():
    _inp = _fwd_setup_inputs()
    _gk = jax.random.fold_in(jax.random.key(int.from_bytes(__import__("os").urandom(4), "little")), 2**31 - 1)
    _shapes = [[1, 384, 384, 96]]
    _dtypes = ['bfloat16']
    _gks = jax.random.split(_gk, len(_shapes))
    _gs = [jax.random.normal(k, s, dtype=jnp.dtype(d)) * 0.05 for k, s, d in zip(_gks, _shapes, _dtypes)]
    _inp["grad_out"] = _gs[0]
    return _inp

def reference(x, w_down, w_up, grad_out):
    _const = dict()
    def _f(*_d):
        return _fwd_reference(**{'x': _d[0], 'w_down': _d[1], 'w_up': _d[2], **_const})
    _out, _vjp = jax.vjp(_f, x, w_down, w_up)
    _grads = _vjp(grad_out)
    _out0 = jnp.asarray(_out)
    return (_out0, *[jnp.asarray(_g) for _g in _grads])
```

```python
import jax
import jax.numpy as jnp
import jax.experimental.pallas as pl
import jax.experimental.pallas.tpu as pltpu

H, W, C, R = 384, 384, 96, 6
LANES, SUB = 128, 8
CT, WT = C // SUB, W // LANES
SLAB = CT * WT * SUB
ROWS = H * SLAB

X_CHUNKS = (32,) * 12
D_CHUNKS = (32,) * 11 + (28, 4)

STREAM_ROWS = 4096
N_STREAMS = ROWS // STREAM_ROWS
STREAMS = 9
N_GROUPS = N_STREAMS // STREAMS
RUN = 128
N_RUNS = STREAM_ROWS // RUN
GROUP_SLABS = H // N_GROUPS
WRITE_VIEW = (N_STREAMS, N_RUNS, RUN, LANES)

F32 = jnp.float32
BF16 = jnp.bfloat16


def _offsets(sizes):
    out, acc = [], 0
    for s in sizes:
        out.append(acc)
        acc += s
    return out


def _tiles(slab):
    return slab.astype(F32).reshape(CT, WT, SUB, LANES)


def _sigmoid(v):
    return 1.0 / (1.0 + jnp.exp(-v))


def _kernel(x_hbm, d_hbm, wd_hbm, wu_hbm,
            out_hbm, dx_hbm, dwd_hbm, dwu_hbm,
            xbuf, dbuf, wd_v, wu_v, dwd_v, dwu_v,
            xsem, dsem, wsem, ssem):
    x_off, d_off = _offsets(X_CHUNKS), _offsets(D_CHUNKS)

    def read(src, buf, sem, off, sizes, i):
        sl = pl.ds(off[i], sizes[i])
        return pltpu.make_async_copy(src.at[sl], buf.at[sl], sem.at[i])

    def read_x(i):
        return read(x_hbm, xbuf, xsem, x_off, X_CHUNKS, i)

    def read_d(i):
        return read(d_hbm, dbuf, dsem, d_off, D_CHUNKS, i)

    xw, dw = xbuf.reshape(WRITE_VIEW), dbuf.reshape(WRITE_VIEW)

    def start_writes(src, dst, sem, group):
        rows = pl.ds(group * STREAMS, STREAMS)

        def body(s, carry):
            pltpu.make_async_copy(src.at[rows, s], dst.at[rows, s], sem).start()
            return carry

        jax.lax.fori_loop(0, N_RUNS, body, 0)

    wd_in = pltpu.make_async_copy(wd_hbm, wd_v, ssem.at[0])
    wu_in = pltpu.make_async_copy(wu_hbm, wu_v, ssem.at[1])
    dwd_out = pltpu.make_async_copy(dwd_v, dwd_hbm, ssem.at[2])
    dwu_out = pltpu.make_async_copy(dwu_v, dwu_hbm, ssem.at[3])

    read_x(0).start()
    wd_in.start()
    wu_in.start()
    for i in range(1, len(X_CHUNKS)):
        read_x(i).start()
    for i in range(len(D_CHUNKS)):
        read_d(i).start()

    eye = (jax.lax.broadcasted_iota(jnp.int32, (C, C), 0)
           == jax.lax.broadcasted_iota(jnp.int32, (C, C), 1))

    def acc_to_row(acc):
        col = jnp.sum(acc.reshape(C, LANES), axis=1, keepdims=True)
        return jnp.sum(jnp.where(eye, col, 0.0), axis=0, keepdims=True)

    def row_to_tiles(row):
        col = jnp.sum(jnp.where(eye, row, 0.0), axis=1, keepdims=True)
        return jnp.broadcast_to(col, (C, LANES)).reshape(CT, 1, SUB, LANES)

    def sum_body(h, acc):
        return acc + jnp.sum(_tiles(xbuf[h]), axis=1)

    acc = jnp.zeros((CT, SUB, LANES), F32)
    for i, n in enumerate(X_CHUNKS):
        read_x(i).wait()
        acc = jax.lax.fori_loop(x_off[i], x_off[i] + n, sum_body, acc)

    wd_in.wait()
    wu_in.wait()
    wd = wd_v[...].astype(F32)
    wu = wu_v[...].astype(F32)
    inv_n = 1.0 / (H * W)
    s = acc_to_row(acc) * inv_n
    z1 = jnp.sum(wd * s, axis=1, keepdims=True)
    sig1 = _sigmoid(z1)
    hid = z1 * sig1
    g = _sigmoid(jnp.sum(wu * hid, axis=0, keepdims=True))
    g_t = row_to_tiles(g)

    def scale_body(h, acc):
        xt = _tiles(xbuf[h])
        acc = acc + jnp.sum(xt * _tiles(dbuf[h]), axis=1)
        xbuf[h] = (xt * g_t).reshape(SLAB, LANES).astype(BF16)
        return acc

    acc = jnp.zeros((CT, SUB, LANES), F32)
    for i, n in enumerate(D_CHUNKS):
        read_d(i).wait()
        if i == len(D_CHUNKS) - 2:
            start_writes(xw, out_hbm, wsem.at[0], 0)
        acc = jax.lax.fori_loop(d_off[i], d_off[i] + n, scale_body, acc)

    dz2 = acc_to_row(acc) * g * (1.0 - g)
    dwu_v[...] = (hid * dz2).astype(BF16)
    dhid = jnp.sum(wu * dz2, axis=1, keepdims=True)
    dz1 = dhid * (sig1 + hid * (1.0 - sig1))
    dwd_v[...] = (dz1 * s).astype(BF16)
    ds_t = row_to_tiles(jnp.sum(wd * dz1, axis=0, keepdims=True) * inv_n)
    dwd_out.start()
    dwu_out.start()

    def dx_body(h, carry):
        dbuf[h] = (_tiles(dbuf[h]) * g_t + ds_t).reshape(SLAB, LANES).astype(BF16)
        return carry

    def compute_dx(group):
        jax.lax.fori_loop(group * GROUP_SLABS, (group + 1) * GROUP_SLABS, dx_body, 0)

    for group in range(1, N_GROUPS):
        start_writes(xw, out_hbm, wsem.at[0], group)
        compute_dx(group - 1)
    start_writes(dw, dx_hbm, wsem.at[1], 0)
    compute_dx(N_GROUPS - 1)
    for group in range(1, N_GROUPS):
        start_writes(dw, dx_hbm, wsem.at[1], group)

    dwd_out.wait()
    dwu_out.wait()
    pltpu.make_async_copy(xw, out_hbm, wsem.at[0]).wait()
    pltpu.make_async_copy(dw, dx_hbm, wsem.at[1]).wait()


def _to_rows(a):
    a = a.reshape(H, WT, LANES, CT, SUB).transpose(0, 3, 1, 4, 2)
    return a.reshape(H, SLAB, LANES)


def _from_rows(a):
    a = a.reshape(H, CT, WT, SUB, LANES).transpose(0, 2, 4, 1, 3)
    return a.reshape(1, H, W, C)


@jax.jit
def pallas_standalone__channel_attn_se__vision_kernel(
    x: jax.Array,
    w_down: jax.Array,
    w_up: jax.Array,
    grad_out: jax.Array,
):
    assert x.shape == (1, H, W, C) and w_down.shape == (C, R) and w_up.shape == (R, C)
    any_spec = pl.BlockSpec(memory_space=pl.ANY)
    big = jax.ShapeDtypeStruct(WRITE_VIEW, BF16)
    small = jax.ShapeDtypeStruct((R, C), BF16)
    out, dx, dwd_t, dwu = pl.pallas_call(
        _kernel,
        in_specs=[any_spec] * 4,
        out_specs=[any_spec] * 4,
        out_shape=[big, big, small, small],
        scratch_shapes=[
            pltpu.VMEM((H, SLAB, LANES), BF16),
            pltpu.VMEM((H, SLAB, LANES), BF16),
            pltpu.VMEM((R, C), BF16),
            pltpu.VMEM((R, C), BF16),
            pltpu.VMEM((R, C), BF16),
            pltpu.VMEM((R, C), BF16),
            pltpu.SemaphoreType.DMA((len(X_CHUNKS),)),
            pltpu.SemaphoreType.DMA((len(D_CHUNKS),)),
            pltpu.SemaphoreType.DMA((2,)),
            pltpu.SemaphoreType.DMA((4,)),
        ],
        compiler_params=pltpu.CompilerParams(
            vmem_limit_bytes=64 * 1024 * 1024,
            disable_bounds_checks=True,
            disable_semaphore_checks=True,
        ),
    )(_to_rows(x), _to_rows(grad_out), w_down.T, w_up)
    return _from_rows(out), _from_rows(dx), dwd_t.T, dwu
```

```python
import jax
import jax.numpy as jnp
import jax.experimental.pallas as pl
import jax.experimental.pallas.tpu as pltpu

H, W, C, R = 384, 384, 96, 6
LANES, SUB = 128, 8
CT, WT = C // SUB, W // LANES
SLAB = CT * WT * SUB
ROWS = H * SLAB

CHUNK = 32
N_CHUNKS = H // CHUNK
TAIL = 4

STREAM_ROWS = 4096
N_STREAMS = ROWS // STREAM_ROWS
STREAMS = 9
N_GROUPS = N_STREAMS // STREAMS
RUN = 128
N_RUNS = STREAM_ROWS // RUN
GROUP_SLABS = H // N_GROUPS
WRITE_VIEW = (N_STREAMS, N_RUNS, RUN, LANES)

F32 = jnp.float32
BF16 = jnp.bfloat16


def _loop(lo, hi, fn):
    def body(i, carry):
        fn(i)
        return carry

    jax.lax.fori_loop(lo, hi, body, 0)


def _tiles(slab):
    return slab.astype(F32).reshape(CT, WT, SUB, LANES)


def _sigmoid(v):
    return 1.0 / (1.0 + jnp.exp(-v))


def _kernel(x_hbm, d_hbm, wd_hbm, wu_hbm,
            out_hbm, dx_hbm, dwd_hbm, dwu_hbm,
            xbuf, dbuf, wd_v, wu_v, dwd_v, dwu_v,
            xsem, dsem, wsem, ssem):
    def read(src, buf, sem, start, size):
        sl = pl.ds(start, size)
        return pltpu.make_async_copy(src.at[sl], buf.at[sl], sem)

    def read_x(i):
        return read(x_hbm, xbuf, xsem.at[i], i * CHUNK, CHUNK)

    def read_d(i):
        return read(d_hbm, dbuf, dsem.at[i], i * CHUNK, CHUNK)

    read_d_head = read(d_hbm, dbuf, dsem.at[N_CHUNKS - 1], H - CHUNK, CHUNK - TAIL)
    read_d_tail = read(d_hbm, dbuf, dsem.at[N_CHUNKS], H - TAIL, TAIL)

    xw, dw = xbuf.reshape(WRITE_VIEW), dbuf.reshape(WRITE_VIEW)

    def start_writes(src, dst, sem, group):
        rows = pl.ds(group * STREAMS, STREAMS)
        _loop(0, N_RUNS, lambda s: pltpu.make_async_copy(
            src.at[rows, s], dst.at[rows, s], sem).start())

    wd_in = pltpu.make_async_copy(wd_hbm, wd_v, ssem.at[0])
    wu_in = pltpu.make_async_copy(wu_hbm, wu_v, ssem.at[1])
    dwd_out = pltpu.make_async_copy(dwd_v, dwd_hbm, ssem.at[2])
    dwu_out = pltpu.make_async_copy(dwu_v, dwu_hbm, ssem.at[3])

    _loop(0, N_CHUNKS, lambda i: read_x(i).start())
    wd_in.start()
    wu_in.start()
    _loop(0, N_CHUNKS - 1, lambda i: read_d(i).start())
    read_d_head.start()
    read_d_tail.start()

    eye = (jax.lax.broadcasted_iota(jnp.int32, (C, C), 0)
           == jax.lax.broadcasted_iota(jnp.int32, (C, C), 1))

    def acc_to_row(acc):
        col = jnp.sum(acc.reshape(C, LANES), axis=1, keepdims=True)
        return jnp.sum(jnp.where(eye, col, 0.0), axis=0, keepdims=True)

    def row_to_tiles(row):
        col = jnp.sum(jnp.where(eye, row, 0.0), axis=1, keepdims=True)
        return jnp.broadcast_to(col, (C, LANES)).reshape(CT, 1, SUB, LANES)

    def sum_body(h, acc):
        return acc + jnp.sum(_tiles(xbuf[h]), axis=1)

    def over_chunk(i, body, acc):
        return jax.lax.fori_loop(0, CHUNK, lambda j, a: body(i * CHUNK + j, a), acc)

    def x_chunk(i, acc):
        read_x(i).wait()
        return over_chunk(i, sum_body, acc)

    zeros = jnp.zeros((CT, SUB, LANES), F32)
    acc = jax.lax.fori_loop(0, N_CHUNKS, x_chunk, zeros)

    wd_in.wait()
    wu_in.wait()
    wd = wd_v[...].astype(F32)
    wu = wu_v[...].astype(F32)
    inv_n = 1.0 / (H * W)
    s = acc_to_row(acc) * inv_n
    z1 = jnp.sum(wd * s, axis=1, keepdims=True)
    sig1 = _sigmoid(z1)
    hid = z1 * sig1
    g = _sigmoid(jnp.sum(wu * hid, axis=0, keepdims=True))
    g_t = row_to_tiles(g)

    def scale_body(h, acc):
        xt = _tiles(xbuf[h])
        acc = acc + jnp.sum(xt * _tiles(dbuf[h]), axis=1)
        xbuf[h] = (xt * g_t).reshape(SLAB, LANES).astype(BF16)
        return acc

    def d_chunk(i, acc):
        read_d(i).wait()
        return over_chunk(i, scale_body, acc)

    acc = jax.lax.fori_loop(0, N_CHUNKS - 1, d_chunk, zeros)
    read_d_head.wait()
    start_writes(xw, out_hbm, wsem.at[0], 0)
    read_d_tail.wait()
    acc = over_chunk(N_CHUNKS - 1, scale_body, acc)

    dz2 = acc_to_row(acc) * g * (1.0 - g)
    dwu_v[...] = (hid * dz2).astype(BF16)
    dhid = jnp.sum(wu * dz2, axis=1, keepdims=True)
    dz1 = dhid * (sig1 + hid * (1.0 - sig1))
    dwd_v[...] = (dz1 * s).astype(BF16)
    ds_t = row_to_tiles(jnp.sum(wd * dz1, axis=0, keepdims=True) * inv_n)
    dwd_out.start()
    dwu_out.start()

    def dx_body(h):
        dbuf[h] = (_tiles(dbuf[h]) * g_t + ds_t).reshape(SLAB, LANES).astype(BF16)

    def compute_dx(group):
        _loop(group * GROUP_SLABS, (group + 1) * GROUP_SLABS, dx_body)

    for group in range(1, N_GROUPS):
        start_writes(xw, out_hbm, wsem.at[0], group)
        compute_dx(group - 1)
    start_writes(dw, dx_hbm, wsem.at[1], 0)
    compute_dx(N_GROUPS - 1)
    for group in range(1, N_GROUPS):
        start_writes(dw, dx_hbm, wsem.at[1], group)

    dwd_out.wait()
    dwu_out.wait()
    pltpu.make_async_copy(xw, out_hbm, wsem.at[0]).wait()
    pltpu.make_async_copy(dw, dx_hbm, wsem.at[1]).wait()


def _to_rows(a):
    a = a.reshape(H, WT, LANES, CT, SUB).transpose(0, 3, 1, 4, 2)
    return a.reshape(H, SLAB, LANES)


def _from_rows(a):
    a = a.reshape(H, CT, WT, SUB, LANES).transpose(0, 2, 4, 1, 3)
    return a.reshape(1, H, W, C)


@jax.jit
def pallas_standalone__channel_attn_se__vision_kernel(
    x: jax.Array,
    w_down: jax.Array,
    w_up: jax.Array,
    grad_out: jax.Array,
):
    assert x.shape == (1, H, W, C) and w_down.shape == (C, R) and w_up.shape == (R, C)
    any_spec = pl.BlockSpec(memory_space=pl.ANY)
    big = jax.ShapeDtypeStruct(WRITE_VIEW, BF16)
    small = jax.ShapeDtypeStruct((R, C), BF16)
    out, dx, dwd_t, dwu = pl.pallas_call(
        _kernel,
        in_specs=[any_spec] * 4,
        out_specs=[any_spec] * 4,
        out_shape=[big, big, small, small],
        scratch_shapes=[
            pltpu.VMEM((H, SLAB, LANES), BF16),
            pltpu.VMEM((H, SLAB, LANES), BF16),
            pltpu.VMEM((R, C), BF16),
            pltpu.VMEM((R, C), BF16),
            pltpu.VMEM((R, C), BF16),
            pltpu.VMEM((R, C), BF16),
            pltpu.SemaphoreType.DMA((N_CHUNKS,)),
            pltpu.SemaphoreType.DMA((N_CHUNKS + 1,)),
            pltpu.SemaphoreType.DMA((2,)),
            pltpu.SemaphoreType.DMA((4,)),
        ],
        compiler_params=pltpu.CompilerParams(
            vmem_limit_bytes=64 * 1024 * 1024,
            disable_bounds_checks=True,
            disable_semaphore_checks=True,
        ),
    )(_to_rows(x), _to_rows(grad_out), w_down.T, w_up)
    return _from_rows(out), _from_rows(dx), dwd_t.T, dwu
```

```python
import jax
import jax.numpy as jnp
from jax import lax
import jax.experimental.pallas as pl
import jax.experimental.pallas.tpu as pltpu

F32, BF16, I32 = jnp.float32, jnp.bfloat16, jnp.int32

H, W, C, R = 384, 384, 96, 6
LANES, SUB = 128, 8
CT, WT = C // SUB, W // LANES
SLAB = CT * WT * SUB

N_STREAMS, N_RUNS, RUN = 27, 64, 64
LOG2_RUNS = 6
VIEW = (N_STREAMS, N_RUNS, RUN, LANES)

GROUPS, WIDTH, STEPS = 3, 9, 32
LAST = 2 * GROUPS - 1
GROUP_SLABS = H // GROUPS
STEP_SLABS = GROUP_SLABS // STEPS
LAST_STEP_SLABS = 2
LOOK = 8
TAIL, TRIGGER = 6, 4
LAST_STEPS = STEPS - TAIL // 2

N_RING, N_PARK = 78, 54
SLOTS, AHEAD = 8, 5
N_TICKS = N_RING - AHEAD
SIDE0 = N_STREAMS * N_RUNS - N_RING - N_PARK
SIDE_SLAB = SIDE0 * RUN // SLAB
LAST_WIDTH = 7
CLOCK_END = LAST * STEPS * WIDTH + LAST_STEPS * LAST_WIDTH
RING_SPAN = (45, CLOCK_END - 28)
PARK_SPAN = (0, CLOCK_END - 28)
FRAC = 14

W_GROUPS = (7, 7, 7, 6)
W_START = tuple(sum(W_GROUPS[:i]) for i in range(len(W_GROUPS)))
W_SLABS = tuple(-(-(o + n) * N_RUNS * RUN // SLAB) for o, n in zip(W_START, W_GROUPS))
W_FIRST = 4


def _last_width(run):
    first = N_STREAMS - WIDTH
    return sum(j * N_RUNS + run < SIDE0 for j in range(first, N_STREAMS))


assert all(_last_width(r) == LAST_WIDTH for r in range(2 * LAST_STEPS))
assert W_SLABS[0] <= GROUP_SLABS and W_SLABS[-2] <= SIDE_SLAB and W_SLABS[-1] == H


def _loop(lo, hi, fn):
    def body(i, carry):
        fn(i)
        return carry

    lax.fori_loop(lo, hi, body, 0)


def _paced(phase, step, span, count, fn):
    rate = -(-(count << FRAC) // (span[1] - span[0]))
    inc = (WIDTH if phase < LAST else LAST_WIDTH) * rate
    pos = step * inc + ((phase * STEPS * WIDTH - span[0]) * rate + (1 << FRAC) - 1)
    _loop(jnp.clip(pos >> FRAC, 0, count), jnp.clip((pos + inc) >> FRAC, 0, count), fn)


def _tiles(slab):
    return slab.astype(F32).reshape(CT, WT, SUB, LANES)


def _slab(tiles):
    return tiles.reshape(SLAB, LANES).astype(BF16)


def _sigmoid(v):
    return 1.0 / (1.0 + jnp.exp(-v))


def _kernel(x_hbm, d_hbm, wd_hbm, wu_hbm,
            out_hbm, dx_hbm, dwd_hbm, dwu_hbm,
            xv, dv, ring, park, wd_v, wu_v, dwd_v, dwu_v,
            read_sem, tail_sem, fill_sem, drain_sem, park_sem, write_sem, small_sem):
    copy = pltpu.make_async_copy
    xs, ds = xv.reshape(H, SLAB, LANES), dv.reshape(H, SLAB, LANES)

    def read(phase, step):
        src, dst = (x_hbm, xv) if phase < GROUPS else (d_hbm, dv)
        idx = (pl.ds(phase % GROUPS * WIDTH, WIDTH if phase < LAST else LAST_WIDTH),
               pl.ds(2 * step, 2))
        return copy(src.at[idx], dst.at[idx], read_sem.at[step & (LOOK - 1)])

    def read_tail(i):
        run = N_RUNS - TAIL + i
        idx = (pl.ds(N_STREAMS - WIDTH, _last_width(run)), run)
        return copy(d_hbm.at[idx], dv.at[idx], tail_sem.at[i])

    def side_run(ref, k):
        j = SIDE0 + k
        return ref.at[j >> LOG2_RUNS, j & (N_RUNS - 1)]

    def ring_fill(k):
        slot = k & (SLOTS - 1)
        return copy(side_run(d_hbm, k), ring.at[slot], fill_sem.at[slot])

    def ring_drain(k):
        slot = k & (SLOTS - 1)
        return copy(ring.at[slot], side_run(dv, k), drain_sem.at[slot])

    def ring_tick(k):
        ring_fill(k).wait()
        ring_drain(k).start()

        @pl.when(k + AHEAD >= SLOTS)
        def _():
            ring_drain(k + AHEAD - SLOTS).wait()

        ring_fill(k + AHEAD).start()

    def park_fill(k):
        src = d_hbm.at[N_STREAMS - 1, N_RUNS - N_PARK + k]
        copy(src, park.at[k], park_sem.at[0]).start()

    parked = (N_STREAMS - 1, pl.ds(N_RUNS - N_PARK, N_PARK))
    park_filled = copy(d_hbm.at[parked], park, park_sem.at[0])
    park_drain = copy(park, dv.at[parked], park_sem.at[1])

    def write(which, group, lo=0, hi=N_RUNS):
        src, dst = (xv, out_hbm) if which == 0 else (dv, dx_hbm)
        rows = pl.ds(W_START[group], W_GROUPS[group])
        _loop(lo, hi, lambda r: copy(
            src.at[rows, r], dst.at[rows, r], write_sem.at[which]).start())

    wd_in = copy(wd_hbm, wd_v, small_sem.at[0])
    wu_in = copy(wu_hbm, wu_v, small_sem.at[1])
    dwd_out = copy(dwd_v, dwd_hbm, small_sem.at[2])
    dwu_out = copy(dwu_v, dwu_hbm, small_sem.at[3])

    _loop(0, LOOK, lambda s: read(0, s).start())
    _loop(0, AHEAD, lambda k: ring_fill(k).start())
    wd_in.start()
    wu_in.start()

    def over_slabs(lo, n, body, acc):
        return lax.fori_loop(0, n, lambda j, a: body(lo + j, a), acc)

    def read_phase(phase, body, slab0, per_step, acc):
        steps = STEPS if phase < LAST else LAST_STEPS

        def step_fn(s, acc):
            read(phase, s).wait()

            @pl.when(s + LOOK < steps)
            def _():
                read(phase, s + LOOK).start()

            if phase < LAST:
                @pl.when(s + LOOK >= steps)
                def _():
                    read(phase + 1, s + LOOK - steps).start()
            else:
                @pl.when(s + LOOK == steps)
                def _():
                    for i in range(TAIL):
                        read_tail(i).start()

            _paced(phase, s, RING_SPAN, N_TICKS, ring_tick)
            _paced(phase, s, PARK_SPAN, N_PARK, park_fill)
            if body is None:
                return acc
            return over_slabs(slab0 + s * per_step, per_step, body, acc)

        return lax.fori_loop(0, steps, step_fn, acc)

    eye = (lax.broadcasted_iota(I32, (C, C), 0) == lax.broadcasted_iota(I32, (C, C), 1))

    def acc_to_row(acc):
        col = jnp.sum(acc.reshape(C, LANES), axis=1, keepdims=True)
        return jnp.sum(jnp.where(eye, col, 0.0), axis=0, keepdims=True)

    def row_to_tiles(row):
        col = jnp.sum(jnp.where(eye, row, 0.0), axis=1, keepdims=True)
        return jnp.broadcast_to(col, (C, LANES)).reshape(CT, 1, SUB, LANES)

    def sum_body(h, acc):
        return acc + jnp.sum(_tiles(xs[h]), axis=1)

    zeros = jnp.zeros((CT, SUB, LANES), F32)
    read_phase(0, None, 0, 0, jnp.int32(0))
    acc = zeros
    for phase in range(1, GROUPS + 1):
        acc = read_phase(phase, sum_body, (phase - 1) * GROUP_SLABS, STEP_SLABS, acc)

    wd_in.wait()
    wu_in.wait()
    wd = wd_v[...].astype(F32)
    wu = wu_v[...].astype(F32)
    inv_n = 1.0 / (H * W)
    mean = acc_to_row(acc) * inv_n
    z1 = jnp.sum(wd * mean, axis=1, keepdims=True)
    sig1 = _sigmoid(z1)
    hid = z1 * sig1
    gate = _sigmoid(jnp.sum(wu * hid, axis=0, keepdims=True))
    gate_t = row_to_tiles(gate)

    def scale_body(h, acc):
        xt = _tiles(xs[h])
        acc = acc + jnp.sum(xt * _tiles(ds[h]), axis=1)
        xs[h] = _slab(xt * gate_t)
        return acc

    acc = read_phase(LAST - 1, scale_body, 0, STEP_SLABS, zeros)
    acc = read_phase(LAST, scale_body, GROUP_SLABS, LAST_STEP_SLABS, acc)
    done = GROUP_SLABS + LAST_STEPS * LAST_STEP_SLABS

    for i in range(TAIL - TRIGGER):
        read_tail(i).wait()
    write(0, 0, 0, W_FIRST)
    for k in range(N_TICKS, N_RING):
        ring_fill(k).wait()
        ring_drain(k).start()
    park_filled.wait()
    park_drain.start()
    write(0, 0, W_FIRST)
    for i in range(TAIL - TRIGGER, TAIL):
        read_tail(i).wait()

    n_w = len(W_GROUPS)
    for group in range(1, n_w - 1):
        upto = W_SLABS[group] if group < n_w - 2 else SIDE_SLAB
        acc = over_slabs(done, upto - done, scale_body, acc)
        done = upto
        write(0, group)
    for k in range(N_RING - SLOTS, N_RING):
        ring_drain(k).wait()
    park_drain.wait()
    acc = over_slabs(done, H - done, scale_body, acc)

    dz2 = acc_to_row(acc) * gate * (1.0 - gate)
    dwu_v[...] = (hid * dz2).astype(BF16)
    dhid = jnp.sum(wu * dz2, axis=1, keepdims=True)
    dz1 = dhid * (sig1 + hid * (1.0 - sig1))
    dwd_v[...] = (dz1 * mean).astype(BF16)
    dmean_t = row_to_tiles(jnp.sum(wd * dz1, axis=0, keepdims=True) * inv_n)
    dwd_out.start()
    dwu_out.start()
    write(0, n_w - 1)

    def dx_body(h):
        ds[h] = _slab(_tiles(ds[h]) * gate_t + dmean_t)

    for group in range(n_w):
        _loop(W_SLABS[group - 1] if group else 0, W_SLABS[group], dx_body)
        write(1, group)

    dwd_out.wait()
    dwu_out.wait()
    copy(xv, out_hbm, write_sem.at[0]).wait()
    copy(dv, dx_hbm, write_sem.at[1]).wait()


def _to_view(a):
    return a.reshape(H, WT, LANES, CT, SUB).transpose(0, 3, 1, 4, 2).reshape(VIEW)


def _from_view(a):
    return a.reshape(H, CT, WT, SUB, LANES).transpose(0, 2, 4, 1, 3).reshape(1, H, W, C)


@jax.jit
def pallas_standalone__channel_attn_se__vision_kernel(
    x: jax.Array,
    w_down: jax.Array,
    w_up: jax.Array,
    grad_out: jax.Array,
):
    assert x.shape == grad_out.shape == (1, H, W, C)
    assert w_down.shape == (C, R) and w_up.shape == (R, C)
    any_spec = pl.BlockSpec(memory_space=pl.ANY)
    big = jax.ShapeDtypeStruct(VIEW, BF16)
    small = jax.ShapeDtypeStruct((R, C), BF16)
    dma_sems = pltpu.SemaphoreType.DMA
    out, dx, dwd_t, dwu = pl.pallas_call(
        _kernel,
        in_specs=[any_spec] * 4,
        out_specs=[any_spec] * 4,
        out_shape=[big, big, small, small],
        scratch_shapes=[
            pltpu.VMEM(VIEW, BF16),
            pltpu.VMEM(VIEW, BF16),
            pltpu.SMEM((SLOTS, RUN, LANES), BF16),
            pltpu.SMEM((N_PARK, RUN, LANES), BF16),
            pltpu.VMEM((R, C), BF16),
            pltpu.VMEM((R, C), BF16),
            pltpu.VMEM((R, C), BF16),
            pltpu.VMEM((R, C), BF16),
            dma_sems((LOOK,)),
            dma_sems((TAIL,)),
            dma_sems((SLOTS,)),
            dma_sems((SLOTS,)),
            dma_sems((2,)),
            dma_sems((2,)),
            dma_sems((4,)),
        ],
        compiler_params=pltpu.CompilerParams(
            vmem_limit_bytes=64 * 1024 * 1024,
            disable_bounds_checks=True,
            disable_semaphore_checks=True,
        ),
    )(_to_view(x), _to_view(grad_out), w_down.T, w_up)
    return _from_view(out), _from_view(dx), dwd_t.T, dwu
```

```python
import jax
import jax.numpy as jnp
from jax import lax
import jax.experimental.pallas as pl
import jax.experimental.pallas.tpu as pltpu

F32, BF16, I32 = jnp.float32, jnp.bfloat16, jnp.int32

H, W, C, R = 384, 384, 96, 6
LANES, SUB = 128, 8
CT, WT = C // SUB, W // LANES
SLAB = CT * WT * SUB

N_STREAMS, N_RUNS, RUN = 27, 256, 16
VIEW = (N_STREAMS, N_RUNS, RUN, LANES)

GROUPS, WIDTH = 3, 9
SPLIT = (3, 6)
LAST = 2 * GROUPS - 1
GROUP_SLABS = H // GROUPS
HALF = N_RUNS // 2
STEPS = 8
TAIL = 16

W_GROUPS = (7, 7, 7, 6)
W_RUNS = 4
W_START = tuple(sum(W_GROUPS[:i]) for i in range(len(W_GROUPS)))
W_SLABS = tuple(-(-(o + n) * N_RUNS * RUN // SLAB) for o, n in zip(W_START, W_GROUPS))

assert W_SLABS[0] <= GROUP_SLABS <= W_SLABS[1] and W_SLABS[-1] == H


def _loop(lo, hi, fn):
    def body(i, carry):
        fn(i)
        return carry

    lax.fori_loop(lo, hi, body, 0)


def _tiles(slab):
    return slab.astype(F32).reshape(CT, WT, SUB, LANES)


def _slab(tiles):
    return tiles.reshape(SLAB, LANES).astype(BF16)


def _sigmoid(v):
    return 1.0 / (1.0 + jnp.exp(-v))


def _kernel(x_hbm, d_hbm, wd_hbm, wu_hbm,
            out_hbm, dx_hbm, dwd_hbm, dwu_hbm,
            xv, dv, wd_v, wu_v, dwd_v, dwu_v,
            group_sem, last_sem, write_sem, small_sem):
    copy = pltpu.make_async_copy
    xs, ds = xv.reshape(H, SLAB, LANES), dv.reshape(H, SLAB, LANES)

    def read(phase, idx, sem):
        src, dst = (x_hbm, xv) if phase < GROUPS else (d_hbm, dv)
        return copy(src.at[idx], dst.at[idx], sem)

    def streams(phase, prio):
        return pl.ds(phase % GROUPS * WIDTH + prio * SPLIT[0], SPLIT[prio])

    def start_reads(phase, lo, n, tail=False):
        def pair(j):
            for prio in (0, 1):
                sem = group_sem.at[phase] if phase < LAST else last_sem.at[prio * (1 + tail)]
                read(phase, (streams(phase, prio), lo + j), sem).start(priority=prio)

        _loop(0, n, pair)

    def wait_group(phase):
        read(phase, pl.ds(phase % GROUPS * WIDTH, WIDTH), group_sem.at[phase]).wait()

    def wait_last(prio, lo, n, sem):
        read(LAST, (streams(LAST, prio), pl.ds(lo, n)), last_sem.at[sem]).wait()

    def start_writes(which, group):
        src, dst = (xv, out_hbm) if which == 0 else (dv, dx_hbm)

        def one(j):
            idx = (pl.ds(W_START[group], W_GROUPS[group]), pl.ds(j * W_RUNS, W_RUNS))
            copy(src.at[idx], dst.at[idx], write_sem.at[which]).start()

        _loop(0, N_RUNS // W_RUNS, one)

    def over_slabs(lo, n, body, acc):
        return lax.fori_loop(0, n, lambda j, a: body(lo + j, a), acc)

    def reads_with(phase, lo, body, slab0, n_slabs, acc):
        runs, slabs = HALF // STEPS, n_slabs // STEPS

        def step(s, acc):
            start_reads(phase, lo + s * runs, runs)
            return over_slabs(slab0 + s * slabs, slabs, body, acc)

        return lax.fori_loop(0, STEPS, step, acc)

    wd_in = copy(wd_hbm, wd_v, small_sem.at[0])
    wu_in = copy(wu_hbm, wu_v, small_sem.at[1])
    dwd_out = copy(dwd_v, dwd_hbm, small_sem.at[2])
    dwu_out = copy(dwu_v, dwu_hbm, small_sem.at[3])

    start_reads(0, 0, N_RUNS)
    wd_in.start()
    wu_in.start()

    eye = (lax.broadcasted_iota(I32, (C, C), 0) == lax.broadcasted_iota(I32, (C, C), 1))

    def acc_to_row(acc):
        col = jnp.sum(acc.reshape(C, LANES), axis=1, keepdims=True)
        return jnp.sum(jnp.where(eye, col, 0.0), axis=0, keepdims=True)

    def row_to_tiles(row):
        col = jnp.sum(jnp.where(eye, row, 0.0), axis=1, keepdims=True)
        return jnp.broadcast_to(col, (C, LANES)).reshape(CT, 1, SUB, LANES)

    def sum_body(h, acc):
        return acc + jnp.sum(_tiles(xs[h]), axis=1)

    zeros = jnp.zeros((CT, SUB, LANES), F32)
    acc = zeros
    for phase in range(1, GROUPS + 1):
        start_reads(phase, 0, HALF)
        wait_group(phase - 1)
        acc = reads_with(phase, HALF, sum_body, (phase - 1) * GROUP_SLABS, GROUP_SLABS, acc)

    wd_in.wait()
    wu_in.wait()
    wd = wd_v[...].astype(F32)
    wu = wu_v[...].astype(F32)
    inv_n = 1.0 / (H * W)
    mean = acc_to_row(acc) * inv_n
    z1 = jnp.sum(wd * mean, axis=1, keepdims=True)
    sig1 = _sigmoid(z1)
    hid = z1 * sig1
    gate = _sigmoid(jnp.sum(wu * hid, axis=0, keepdims=True))
    gate_t = row_to_tiles(gate)

    def scale_body(h, acc):
        xt = _tiles(xs[h])
        acc = acc + jnp.sum(xt * _tiles(ds[h]), axis=1)
        xs[h] = _slab(xt * gate_t)
        return acc

    start_reads(LAST - 1, 0, HALF)
    wait_group(LAST - 2)
    acc = reads_with(LAST - 1, HALF, scale_body, 0, GROUP_SLABS // 2, zeros)
    acc = reads_with(LAST, 0, scale_body, GROUP_SLABS // 2, GROUP_SLABS // 2, acc)
    wait_group(LAST - 1)
    start_reads(LAST, HALF, HALF - TAIL)
    start_reads(LAST, N_RUNS - TAIL, TAIL, tail=True)

    wait_last(1, 0, N_RUNS - TAIL, 1)
    start_writes(0, 0)
    wait_last(0, 0, N_RUNS, 0)
    wait_last(1, N_RUNS - TAIL, TAIL, 2)

    n_w = len(W_GROUPS)
    done = GROUP_SLABS
    for group in range(1, n_w):
        acc = over_slabs(done, W_SLABS[group] - done, scale_body, acc)
        done = W_SLABS[group]
        start_writes(0, group)

    dz2 = acc_to_row(acc) * gate * (1.0 - gate)
    dwu_v[...] = (hid * dz2).astype(BF16)
    dhid = jnp.sum(wu * dz2, axis=1, keepdims=True)
    dz1 = dhid * (sig1 + hid * (1.0 - sig1))
    dwd_v[...] = (dz1 * mean).astype(BF16)
    dmean_t = row_to_tiles(jnp.sum(wd * dz1, axis=0, keepdims=True) * inv_n)
    dwd_out.start()
    dwu_out.start()

    def dx_body(h):
        ds[h] = _slab(_tiles(ds[h]) * gate_t + dmean_t)

    for group in range(n_w):
        _loop(W_SLABS[group - 1] if group else 0, W_SLABS[group], dx_body)
        start_writes(1, group)

    dwd_out.wait()
    dwu_out.wait()
    copy(xv, out_hbm, write_sem.at[0]).wait()
    copy(dv, dx_hbm, write_sem.at[1]).wait()


def _to_view(a):
    return a.reshape(H, WT, LANES, CT, SUB).transpose(0, 3, 1, 4, 2).reshape(VIEW)


def _from_view(a):
    return a.reshape(H, CT, WT, SUB, LANES).transpose(0, 2, 4, 1, 3).reshape(1, H, W, C)


@jax.jit
def pallas_standalone__channel_attn_se__vision_kernel(
    x: jax.Array,
    w_down: jax.Array,
    w_up: jax.Array,
    grad_out: jax.Array,
):
    assert x.shape == grad_out.shape == (1, H, W, C)
    assert w_down.shape == (C, R) and w_up.shape == (R, C)
    any_spec = pl.BlockSpec(memory_space=pl.ANY)
    big = jax.ShapeDtypeStruct(VIEW, BF16)
    small = jax.ShapeDtypeStruct((R, C), BF16)
    dma_sems = pltpu.SemaphoreType.DMA
    out, dx, dwd_t, dwu = pl.pallas_call(
        _kernel,
        in_specs=[any_spec] * 4,
        out_specs=[any_spec] * 4,
        out_shape=[big, big, small, small],
        scratch_shapes=[
            pltpu.VMEM(VIEW, BF16),
            pltpu.VMEM(VIEW, BF16),
            pltpu.VMEM((R, C), BF16),
            pltpu.VMEM((R, C), BF16),
            pltpu.VMEM((R, C), BF16),
            pltpu.VMEM((R, C), BF16),
            dma_sems((LAST,)),
            dma_sems((3,)),
            dma_sems((2,)),
            dma_sems((4,)),
        ],
        compiler_params=pltpu.CompilerParams(
            vmem_limit_bytes=64 * 1024 * 1024,
            disable_bounds_checks=True,
            disable_semaphore_checks=True,
        ),
    )(_to_view(x), _to_view(grad_out), w_down.T, w_up)
    return _from_view(out), _from_view(dx), dwd_t.T, dwu
```

```python
import jax
import jax.numpy as jnp
from jax import lax
import jax.experimental.pallas as pl
import jax.experimental.pallas.tpu as pltpu

F32, BF16, I32 = jnp.float32, jnp.bfloat16, jnp.int32

H, W, C, R = 384, 384, 96, 6
LANES, SUB = 128, 8
CT, WT = C // SUB, W // LANES
SLAB = CT * WT * SUB

N_STREAMS, N_RUNS, RUN = 27, 256, 16
VIEW = (N_STREAMS, N_RUNS, RUN, LANES)

R_GROUPS = ((2, 12), (2, 11))
R_START = (0, sum(R_GROUPS[0]))
R_SLABS = (R_START[1] * N_RUNS * RUN // SLAB, H)
LAST = 3
LAG = 56
HEAD_SLABS = 128
TAIL = 10

W_GROUPS = (7, 7, 7, 6)
W_RUNS = 4
W_START = tuple(sum(W_GROUPS[:i]) for i in range(len(W_GROUPS)))
W_SLABS = tuple(-(-(o + n) * N_RUNS * RUN // SLAB) for o, n in zip(W_START, W_GROUPS))

assert W_SLABS[0] <= HEAD_SLABS <= min(R_SLABS[0], W_SLABS[1]) and W_SLABS[-1] == H
assert LAG + R_SLABS[0] <= N_RUNS and LAG + HEAD_SLABS <= N_RUNS - TAIL


def _loop(lo, hi, fn):
    def body(i, carry):
        fn(i)
        return carry

    lax.fori_loop(lo, hi, body, 0)


def _tiles(slab):
    return slab.astype(F32).reshape(CT, WT, SUB, LANES)


def _slab(tiles):
    return tiles.reshape(SLAB, LANES).astype(BF16)


def _sigmoid(v):
    return 1.0 / (1.0 + jnp.exp(-v))


def _kernel(x_hbm, d_hbm, wd_hbm, wu_hbm,
            out_hbm, dx_hbm, dwd_hbm, dwu_hbm,
            xv, dv, wd_v, wu_v, dwd_v, dwu_v,
            group_sem, last_sem, write_sem, small_sem):
    copy = pltpu.make_async_copy
    xs, ds = xv.reshape(H, SLAB, LANES), dv.reshape(H, SLAB, LANES)

    def read(phase, idx, sem):
        src, dst = (x_hbm, xv) if phase < 2 else (d_hbm, dv)
        return copy(src.at[idx], dst.at[idx], sem)

    def streams(phase, prio):
        split = R_GROUPS[phase % 2]
        return pl.ds(R_START[phase % 2] + prio * split[0], split[prio])

    def start_run(phase, run, tail=False):
        for prio in (0, 1):
            sem = group_sem.at[phase] if phase < LAST else last_sem.at[prio * (1 + tail)]
            read(phase, (streams(phase, prio), run), sem).start(priority=prio)

    def start_reads(phase, lo, hi, tail=False):
        _loop(lo, hi, lambda run: start_run(phase, run, tail))

    def wait_group(phase):
        group = pl.ds(R_START[phase % 2], sum(R_GROUPS[phase % 2]))
        read(phase, group, group_sem.at[phase]).wait()

    def wait_last(prio, lo, n, sem):
        read(LAST, (streams(LAST, prio), pl.ds(lo, n)), last_sem.at[sem]).wait()

    def start_writes(which, group):
        src, dst = (xv, out_hbm) if which == 0 else (dv, dx_hbm)

        def one(j):
            idx = (pl.ds(W_START[group], W_GROUPS[group]), pl.ds(j * W_RUNS, W_RUNS))
            copy(src.at[idx], dst.at[idx], write_sem.at[which]).start()

        _loop(0, N_RUNS // W_RUNS, one)

    def read_phase(phase, n_runs, body, slab_lo, slab_hi, acc):
        def step(h, acc):
            start_run(phase, h + (LAG - slab_lo))
            return body(h, acc)

        start_reads(phase, 0, LAG)
        wait_group(phase - 1)
        acc = lax.fori_loop(slab_lo, slab_hi, step, acc)
        start_reads(phase, LAG + slab_hi - slab_lo, n_runs)
        return acc

    wd_in = copy(wd_hbm, wd_v, small_sem.at[0])
    wu_in = copy(wu_hbm, wu_v, small_sem.at[1])
    dwd_out = copy(dwd_v, dwd_hbm, small_sem.at[2])
    dwu_out = copy(dwu_v, dwu_hbm, small_sem.at[3])

    start_reads(0, 0, N_RUNS)
    wd_in.start()
    wu_in.start()

    eye = (lax.broadcasted_iota(I32, (C, C), 0) == lax.broadcasted_iota(I32, (C, C), 1))

    def acc_to_row(acc):
        col = jnp.sum(acc.reshape(C, LANES), axis=1, keepdims=True)
        return jnp.sum(jnp.where(eye, col, 0.0), axis=0, keepdims=True)

    def row_to_tiles(row):
        col = jnp.sum(jnp.where(eye, row, 0.0), axis=1, keepdims=True)
        return jnp.broadcast_to(col, (C, LANES)).reshape(CT, 1, SUB, LANES)

    def sum_body(h, acc):
        return acc + jnp.sum(_tiles(xs[h]), axis=1)

    zeros = jnp.zeros((CT, SUB, LANES), F32)
    acc = read_phase(1, N_RUNS, sum_body, 0, R_SLABS[0], zeros)
    acc = read_phase(2, N_RUNS, sum_body, R_SLABS[0], H, acc)

    wd_in.wait()
    wu_in.wait()
    wd = wd_v[...].astype(F32)
    wu = wu_v[...].astype(F32)
    inv_n = 1.0 / (H * W)
    mean = acc_to_row(acc) * inv_n
    z1 = jnp.sum(wd * mean, axis=1, keepdims=True)
    sig1 = _sigmoid(z1)
    hid = z1 * sig1
    gate = _sigmoid(jnp.sum(wu * hid, axis=0, keepdims=True))
    gate_t = row_to_tiles(gate)

    def scale_body(h, acc):
        xt = _tiles(xs[h])
        acc = acc + jnp.sum(xt * _tiles(ds[h]), axis=1)
        xs[h] = _slab(xt * gate_t)
        return acc

    acc = read_phase(LAST, N_RUNS - TAIL, scale_body, 0, HEAD_SLABS, zeros)
    start_reads(LAST, N_RUNS - TAIL, N_RUNS, tail=True)

    wait_last(1, 0, N_RUNS - TAIL, 1)
    start_writes(0, 0)
    wait_last(0, 0, N_RUNS, 0)
    wait_last(1, N_RUNS - TAIL, TAIL, 2)

    n_w = len(W_GROUPS)
    done = HEAD_SLABS
    for group in range(1, n_w):
        acc = lax.fori_loop(done, W_SLABS[group], scale_body, acc)
        done = W_SLABS[group]
        start_writes(0, group)

    dz2 = acc_to_row(acc) * gate * (1.0 - gate)
    dwu_v[...] = (hid * dz2).astype(BF16)
    dhid = jnp.sum(wu * dz2, axis=1, keepdims=True)
    dz1 = dhid * (sig1 + hid * (1.0 - sig1))
    dwd_v[...] = (dz1 * mean).astype(BF16)
    dmean_t = row_to_tiles(jnp.sum(wd * dz1, axis=0, keepdims=True) * inv_n)
    dwd_out.start()
    dwu_out.start()

    def dx_body(h):
        ds[h] = _slab(_tiles(ds[h]) * gate_t + dmean_t)

    for group in range(n_w):
        _loop(W_SLABS[group - 1] if group else 0, W_SLABS[group], dx_body)
        start_writes(1, group)

    dwd_out.wait()
    dwu_out.wait()
    copy(xv, out_hbm, write_sem.at[0]).wait()
    copy(dv, dx_hbm, write_sem.at[1]).wait()


def _to_view(a):
    return a.reshape(H, WT, LANES, CT, SUB).transpose(0, 3, 1, 4, 2).reshape(VIEW)


def _from_view(a):
    return a.reshape(H, CT, WT, SUB, LANES).transpose(0, 2, 4, 1, 3).reshape(1, H, W, C)


@jax.jit
def pallas_standalone__channel_attn_se__vision_kernel(
    x: jax.Array,
    w_down: jax.Array,
    w_up: jax.Array,
    grad_out: jax.Array,
):
    assert x.shape == grad_out.shape == (1, H, W, C)
    assert w_down.shape == (C, R) and w_up.shape == (R, C)
    any_spec = pl.BlockSpec(memory_space=pl.ANY)
    big = jax.ShapeDtypeStruct(VIEW, BF16)
    small = jax.ShapeDtypeStruct((R, C), BF16)
    dma_sems = pltpu.SemaphoreType.DMA
    out, dx, dwd_t, dwu = pl.pallas_call(
        _kernel,
        in_specs=[any_spec] * 4,
        out_specs=[any_spec] * 4,
        out_shape=[big, big, small, small],
        scratch_shapes=[
            pltpu.VMEM(VIEW, BF16),
            pltpu.VMEM(VIEW, BF16),
            pltpu.VMEM((R, C), BF16),
            pltpu.VMEM((R, C), BF16),
            pltpu.VMEM((R, C), BF16),
            pltpu.VMEM((R, C), BF16),
            dma_sems((LAST,)),
            dma_sems((3,)),
            dma_sems((2,)),
            dma_sems((4,)),
        ],
        compiler_params=pltpu.CompilerParams(
            vmem_limit_bytes=64 * 1024 * 1024,
            disable_bounds_checks=True,
            disable_semaphore_checks=True,
        ),
    )(_to_view(x), _to_view(grad_out), w_down.T, w_up)
    return _from_view(out), _from_view(dx), dwd_t.T, dwu
```
